```python
import jax
import jax.numpy as jnp

def _softmax(x, axis=-1):
    return jax.nn.softmax(x, axis=axis)
def _gelu(x):
    return jax.nn.gelu(x, approximate=True)
def _silu(x):
    return jax.nn.silu(x)
def _sigmoid(x):
    return jax.nn.sigmoid(x)
def _layernorm(x, axis=-1, eps=1e-5):
    m = jnp.mean(x, axis=axis, keepdims=True)
    v = jnp.var(x, axis=axis, keepdims=True)
    return (x - m) / jnp.sqrt(v + eps)
def _scatter_add(tgt, idx, src, axis=0):
    return tgt.at[idx].add(src)
def _segment_sum(src, seg, n):
    return jax.ops.segment_sum(src, seg, n)
class _Rng:
    def __init__(self, key):
        self._k = key
    def _next(self):
        self._k, sub = jax.random.split(self._k)
        return sub
    def normal(self, shape):
        return jax.random.normal(self._next(), shape, dtype=jnp.bfloat16)
    def randint(self, lo, hi, shape):
        return jax.random.randint(self._next(), shape, lo, hi, dtype=jnp.int32)
    def uniform(self, shape, lo=0.0, hi=1.0):
        return jax.random.uniform(self._next(), shape, jnp.bfloat16, lo, hi)
    def permutation(self, n):
        return jax.random.permutation(self._next(), n)


kernel_name = 'concat_heads__compressed_kv_cla__spectral_gfnet__prompt'

def setup_inputs():
    _rng = _Rng(jax.random.key(int.from_bytes(__import__("os").urandom(4), "little")))
    _w = (lambda a: (lambda t: t.astype(jnp.bfloat16) if jnp.issubdtype(t.dtype, jnp.floating) else t)(jnp.asarray(a)))
    def _A_setup():
        B, H, Sq, Sk, D, M = 1, 32, 2048, 2048, 128, 1024
        Dc = 4 * D
        return {
            "x": _w((lambda *s: _rng.normal(s) * 0.05)(B, Sq, M)),
            "c_kv": _w((lambda *s: _rng.normal(s) * 0.05)(B, Sk, Dc)),
            "w_q": _w((lambda *s: _rng.normal(s) * 0.05)(M, H, D) * (M ** -0.5)),
            "w_uk": _w((lambda *s: _rng.normal(s) * 0.05)(Dc, H, D) * (Dc ** -0.5)),
            "w_uv": _w((lambda *s: _rng.normal(s) * 0.05)(Dc, H, D) * (Dc ** -0.5)),
            "w_o": _w((lambda *s: _rng.normal(s) * 0.05)(H, D, M) * ((H * D) ** -0.5)),
        }
    _A_in = _A_setup()

    def _B_setup():
        B, S, D = 1, 2048, 1024
        Df = D // 2 + 1
        return {
            "x": _w((lambda *s: _rng.normal(s) * 0.05)(B, S, D)),
            "w_r": _w((lambda *s: _rng.normal(s) * 0.05)(S, Df) * 0.02),
            "w_i": _w((lambda *s: _rng.normal(s) * 0.05)(S, Df) * 0.02),
        }
    _B_in = _B_setup()

    return {
        "A_x": _A_in["x"],
        "A_c_kv": _A_in["c_kv"],
        "A_w_q": _A_in["w_q"],
        "A_w_uk": _A_in["w_uk"],
        "A_w_uv": _A_in["w_uv"],
        "A_w_o": _A_in["w_o"],
        "B_x": _B_in["x"],
        "B_w_r": _B_in["w_r"],
        "B_w_i": _B_in["w_i"],
    }

def reference(A_x, A_c_kv, A_w_q, A_w_uk, A_w_uv, A_w_o, B_x, B_w_r, B_w_i):
    def _A_ref(x, c_kv, w_q, w_uk, w_uv, w_o):
        B, Sq, M = x.shape[0], x.shape[1], x.shape[2]
        Sk = c_kv.shape[1]
        H, D = w_q.shape[1], w_q.shape[2]
        q = jnp.einsum("bqm,mhd->bhqd", x, w_q)
        k = jnp.einsum("bkc,chd->bhkd", c_kv, w_uk)
        v = jnp.einsum("bkc,chd->bhkd", c_kv, w_uv)
        scores = jnp.einsum("bhqd,bhkd->bhqk", q, k) * (D ** -0.5)
        off = Sk - Sq
        qi = jnp.arange(Sq)[:, None]
        kj = jnp.arange(Sk)[None, :]
        cmask = kj <= (qi + off)
        scores = jnp.where(cmask[None, None], scores, -1e9)
        p = _softmax(scores, axis=-1)
        ctx = jnp.einsum("bhqk,bhkd->bhqd", p, v)
        return jnp.einsum("bhqd,hdm->bqm", ctx, w_o)

    def _B_ref(x, w_r, w_i):
        B, S, D = x.shape
        X = (lambda x, axes=(-2,-1): jnp.fft.rfft2(x.astype(jnp.float32), axes=axes))(x, axes=(-2, -1))
        W = w_r + 1j * w_i
        X = X * W
        y = (lambda x, s, axes=(-2,-1): jnp.fft.irfft2(x, s=s, axes=axes).astype(jnp.bfloat16))(X, (S, D), axes=(-2, -1))
        return y

    a = _A_ref(A_x, A_c_kv, A_w_q, A_w_uk, A_w_uv, A_w_o)
    b = _B_ref(B_x, B_w_r, B_w_i)
    return jnp.concatenate([a, b], axis=-1)
```

```python
import jax
import jax.numpy as jnp
import ml_dtypes
import numpy as np
from jax import lax
from jax.experimental import pallas as pl
from jax.experimental.pallas import tpu as pltpu

S = 2048
D = 128
M = 1024
DC = 512
H = 32
NP = H // 2
BQ = 256
CK = 512
NR = 528

F32 = jnp.float32
BF = jnp.bfloat16
U32 = jnp.uint32
NT = (((1,), (1,)), ((), ()))
LOG2E = 1.4426950408889634
C45 = float(np.sqrt(0.5))
HI = np.uint32(0xFFFF0000)


def _k1d(q, h):
    if q == 0:
        return 0 if h == 0 else 4
    return q if h == 0 else 8 - q


def _bf(a):
    return np.asarray(a, np.float32).astype(ml_dtypes.bfloat16)


def _dft_consts():
    b = np.arange(128)[:, None]
    k2 = np.arange(64)[None, :]
    Mf = np.zeros((4, 256, 256))
    Mi = np.zeros((4, 256, 256))
    for q in range(4):
        Ta = np.exp(-2j * np.pi * b * (_k1d(q, 0) + 8 * k2) / 1024.0)
        Tb = np.exp(-2j * np.pi * b * (_k1d(q, 1) + 8 * k2) / 1024.0)
        if q == 0:
            Mf[q, :128, 0:64] = Ta.real
            Mf[q, 128:, 64:128] = Tb.real
            Mf[q, :128, 128:192] = Ta.imag
            Mf[q, 128:, 192:256] = Tb.imag
            w = np.full(256, 2.0)
            w[0] = 1.0
            w[128] = 0.0
            Mi[q] = (Mf[q].T * w[:, None]) / 1024.0
        else:
            Mf[q, :128, 0:64] = Ta.real
            Mf[q, 128:, 0:64] = -Ta.imag
            Mf[q, :128, 64:128] = Tb.real
            Mf[q, 128:, 64:128] = Tb.imag
            Mf[q, :128, 128:192] = Ta.imag
            Mf[q, 128:, 128:192] = Ta.real
            Mf[q, :128, 192:256] = Tb.imag
            Mf[q, 128:, 192:256] = -Tb.real
            Mi[q] = Mf[q].T * 2.0 / 1024.0
    MfT = np.transpose(Mf, (0, 2, 1)).copy()
    Ny = np.zeros((16, 256))
    Ny[0, :128] = (-1.0) ** np.arange(128)
    d1 = np.arange(128)[:, None]
    k1 = np.arange(128)[None, :]
    F = np.zeros((16, 256, 256))
    Fh = np.zeros((16, 256, 256))
    for d2 in range(16):
        f = np.exp(-2j * np.pi * (d1 * k1 / 128.0 + d2 * k1 / 2048.0))
        F[d2] = np.block([[f.real, f.imag], [-f.imag, f.real]])
        h = np.conj(f) / 2048.0
        Fh[d2] = np.block([[h.real, -h.imag], [h.imag, h.real]])
    Mf0 = np.concatenate([MfT[0], Ny], axis=0)
    return _bf(Mf0), _bf(MfT), _bf(Mi), _bf(F), _bf(Fh)


def _lo(a):
    return pltpu.bitcast(a << 16, F32)


def _hi(a):
    return pltpu.bitcast(a & HI, F32)


def _unpack(a):
    return _lo(a).astype(BF), _hi(a).astype(BF)


def _tilered(s, op):
    m = s[:, :128]
    for j in range(1, s.shape[1] // 128):
        m = op(m, s[:, j * 128:(j + 1) * 128])
    return m


def _twiddle(xr, xi, k):
    k %= 16
    if k == 0:
        return xr, xi
    if k == 4:
        return -xi, xr
    if k == 8:
        return -xr, -xi
    if k == 12:
        return xi, -xr
    if k == 2:
        return (xr - xi) * C45, (xr + xi) * C45
    if k == 6:
        return (xr + xi) * (-C45), (xr - xi) * C45
    if k == 10:
        return (xi - xr) * C45, (xr + xi) * (-C45)
    if k == 14:
        return (xr + xi) * C45, (xi - xr) * C45
    c = float(np.cos(2 * np.pi * k / 16))
    s = float(np.sin(2 * np.pi * k / 16))
    return xr * c - xi * s, xr * s + xi * c


def _dft4(a, sign):
    (r0, i0), (r1, i1), (r2, i2), (r3, i3) = a
    sr, si = r0 + r2, i0 + i2
    dr, di = r0 - r2, i0 - i2
    tr, ti = r1 + r3, i1 + i3
    ur, ui = r1 - r3, i1 - i3
    o0 = (sr + tr, si + ti)
    o2 = (sr - tr, si - ti)
    if sign < 0:
        o1 = (dr + ui, di - ur)
        o3 = (dr - ui, di + ur)
    else:
        o1 = (dr - ui, di + ur)
        o3 = (dr + ui, di - ur)
    return [o0, o1, o2, o3]


def _dft16(a, sign):
    t = [[None] * 4 for _ in range(4)]
    for n2 in range(4):
        o = _dft4([a[4 * n1 + n2] for n1 in range(4)], sign)
        for k1 in range(4):
            t[k1][n2] = _twiddle(o[k1][0], o[k1][1], sign * n2 * k1)
    out = [None] * 16
    for k1 in range(4):
        o = _dft4(t[k1], sign)
        for k2 in range(4):
            out[k1 + 4 * k2] = o[k2]
    return out


def _pack_pair(a, b):
    ua = pltpu.bitcast(a.astype(BF).astype(F32), U32)
    ub = pltpu.bitcast(b.astype(BF).astype(F32), U32)
    return (ua >> 16) | (ub & HI)


def _att_pair(slot, x_ref, c_ref, acc_ref, q_s, k_s, v_s, wq_b, wuk_b, wuv_b, wo_b):
    wq = jnp.concatenate(_unpack(wq_b[slot]), axis=1)
    wkv = jnp.concatenate(_unpack(wuk_b[slot]) + _unpack(wuv_b[slot]), axis=1)
    wo = wo_b[slot]
    qscale = (D ** -0.5) * LOG2E
    n = S // BQ

    def proj(i):
        r = slice(i * BQ, (i + 1) * BQ)
        q = jnp.dot(x_ref[r, :], wq, preferred_element_type=F32)
        q_s[r, :] = (q * qscale).astype(BF)
        kv = jnp.dot(c_ref[r, :], wkv, preferred_element_type=F32).astype(BF)
        k_s[r, :] = kv[:, :256]
        v_s[r, :] = kv[:, 256:]

    rr = lax.broadcasted_iota(jnp.int32, (128, 128), 0)
    cc = lax.broadcasted_iota(jnp.int32, (128, 128), 1)
    tri = cc <= rr
    NEG = -1e30

    work = []
    for i in range(n):
        for h in range(2):
            kv = BQ * (i + 1) - 128
            c0 = 0
            while c0 < kv:
                w = min(CK, kv - c0)
                work.append((h, i, "f", c0, w, c0 == 0))
                c0 += w
            work.append((h, i, "b", kv, 128, False))
    G = len(work)

    def qk(g):
        h, i, kind, c0, w, first = work[g]
        hs = slice(h * 128, (h + 1) * 128)
        if kind == "f":
            s = lax.dot_general(q_s[i * BQ:(i + 1) * BQ, hs], k_s[c0:c0 + w, hs], NT,
                                preferred_element_type=F32)
            if c0 + w == BQ * (i + 1) - 128:
                top = jnp.where(tri, s[:128, w - 128:], NEG)
                lastt = jnp.concatenate([top, s[128:, w - 128:]], axis=0)
                s = jnp.concatenate([s[:, :w - 128], lastt], axis=1) if w > 128 else lastt
            return s
        s = lax.dot_general(q_s[i * BQ + 128:(i + 1) * BQ, hs], k_s[c0:c0 + w, hs], NT,
                            preferred_element_type=F32)
        return jnp.where(tri, s, NEG)

    st = {}
    ctxs = {}

    def smpv(g, s):
        h, i, kind, c0, w, first = work[g]
        hs = slice(h * 128, (h + 1) * 128)
        vv = v_s[c0:c0 + w, hs]
        mc = jnp.max(_tilered(s, jnp.maximum), axis=1, keepdims=True)
        if kind == "f":
            if first:
                m = mc
                pp = jnp.exp2(s - m)
                l = _tilered(pp, jnp.add)
                o = jnp.dot(pp.astype(BF), vv, preferred_element_type=F32)
            else:
                m0, l0, o0 = st[(h, i)]
                m = jnp.maximum(m0, mc)
                alpha = jnp.exp2(m0 - m)
                pp = jnp.exp2(s - m)
                l = l0 * alpha + _tilered(pp, jnp.add)
                o = o0 * alpha + jnp.dot(pp.astype(BF), vv, preferred_element_type=F32)
            st[(h, i)] = (m, l, o)
        else:
            m0, l0, o0 = st.pop((h, i))
            mb = jnp.maximum(m0[128:], mc)
            alpha = jnp.exp2(m0[128:] - mb)
            pp = jnp.exp2(s - mb)
            lb = l0[128:] * alpha + pp
            ob = o0[128:] * alpha + jnp.dot(pp.astype(BF), vv, preferred_element_type=F32)
            l = jnp.concatenate([l0[:128], lb], axis=0)
            o = jnp.concatenate([o0[:128], ob], axis=0)
            lsum = jnp.sum(l, axis=1, keepdims=True)
            ctxs[(h, i)] = (o * pltpu.reciprocal(lsum, approx=False)).astype(BF)

    def op(i):
        ctx = jnp.concatenate([ctxs.pop((0, i)), ctxs.pop((1, i))], axis=1)
        acc_ref[i * BQ:(i + 1) * BQ, :] += jnp.dot(ctx, wo, preferred_element_type=F32)

    proj(0)
    proj(1)
    nproj = 2
    ss = {0: qk(0)}
    pend = []
    for g in range(G):
        if g + 1 < G:
            h, i, kind, c0, w, first = work[g + 1]
            if first and h == 0 and nproj < n and i + 1 >= nproj:
                proj(nproj)
                nproj += 1
            ss[g + 1] = qk(g + 1)
        smpv(g, ss.pop(g))
        h, i, kind = work[g][:3]
        if kind == "b" and h == 1:
            pend.append((g, i))
        while pend and pend[0][0] + 1 <= g:
            op(pend.pop(0)[1])
    for _, i in pend:
        op(i)


def _b_fwd(jj, xb, mf0_ref, mft_ref, f_ref, xs):
    w = [xb[jj, :, 128 * a:128 * (a + 1)] for a in range(8)]
    for e in range(2):
        d2 = 2 * jj + e
        xa = [(_lo if e == 0 else _hi)(v) for v in w]
        u = [xa[a] - xa[a + 4] for a in range(4)]
        ee = [xa[a] + xa[a + 4] for a in range(4)]
        t0 = ee[0] + ee[2]
        t1 = ee[1] + ee[3]
        Y0 = t0 + t1
        Y4 = t0 - t1
        d = (u[1] - u[3]) * C45
        s = (u[1] + u[3]) * C45
        ins = [(Y0, Y4), (u[0] + d, -(u[2] + s)), (ee[0] - ee[2], ee[3] - ee[1]), (u[0] - d, u[2] - s)]
        zr = []
        zi = []
        for q in range(4):
            r = jnp.concatenate([ins[q][0].astype(BF), ins[q][1].astype(BF)], axis=1)
            lhs = mf0_ref[...] if q == 0 else mft_ref[q]
            z = lax.dot_general(lhs, r, NT, preferred_element_type=F32)
            zr.append(z[:128].astype(BF))
            zi.append(z[128:256].astype(BF))
            if q == 0:
                ny = z[256:272].astype(BF)
        zr = jnp.concatenate(zr + [ny], axis=0)
        zi = jnp.concatenate(zi + [jnp.zeros((16, 128), BF)], axis=0)
        xs[d2] = jnp.dot(jnp.concatenate([zr, zi], axis=1), f_ref[d2], preferred_element_type=F32)


def _b_mid_group(r, wsel, xs, us):
    a = [(xs[d, r, 0:128], xs[d, r, 128:256]) for d in range(16)]
    X = _dft16(a, -1)
    Y = []
    for k2 in range(16):
        wr, wi = wsel(k2)
        xr, xi = X[k2]
        Y.append((xr * wr - xi * wi, xr * wi + xi * wr))
    U = _dft16(Y, +1)
    for d in range(16):
        us[d, r, 0:128] = U[d][0].astype(BF)
        us[d, r, 128:256] = U[d][1].astype(BF)


def _b_mid(xs, us, wr_b, wi_b, wrn, win):
    for q in range(4):
        for h in range(2):
            kk = _k1d(q, h)
            j = kk // 2
            sel = _lo if kk % 2 == 0 else _hi

            def body(gg, carry, q=q, h=h, j=j, sel=sel):
                r = pl.ds(pl.multiple_of(128 * q + 64 * h + 16 * gg, 16), 16)
                rows = pl.ds(j + 64 * gg, 16, stride=4)
                _b_mid_group(r, lambda k2: (sel(wr_b[k2, rows, :]), sel(wi_b[k2, rows, :])), xs, us)
                return carry

            lax.fori_loop(0, 4, body, 0)
    _b_mid_group(
        slice(512, 528),
        lambda k2: (jnp.broadcast_to(wrn[0:1, 128 * k2:128 * (k2 + 1)].astype(F32), (16, 128)),
                    jnp.broadcast_to(win[0:1, 128 * k2:128 * (k2 + 1)].astype(F32), (16, 128))),
        xs, us)


def _b_inv(jj, us, fh_ref, mi_ref, ob):
    sgn = jnp.where(lax.broadcasted_iota(jnp.int32, (128, 128), 1) % 2 == 0,
                    1.0 / 1024, -1.0 / 1024).astype(F32)
    ys = []
    for e in range(2):
        d2 = 2 * jj + e
        fh = fh_ref[d2]
        V = []
        for q in range(4):
            o = lax.dot_general(fh, us[d2, 128 * q:128 * (q + 1), :], NT, preferred_element_type=F32)
            lhs = jnp.concatenate([o[:128].astype(BF), o[128:].astype(BF)], axis=1)
            V.append(jnp.dot(lhs, mi_ref[q], preferred_element_type=F32))
        on = lax.dot_general(fh[:128], us[d2, 512:528, :], NT, preferred_element_type=F32)
        ny = on[:, 0:1]
        V0 = V[0][:, :128] + ny * sgn
        V4 = V[0][:, 128:]
        A = [None] + [V[q][:, :128] for q in (1, 2, 3)]
        B = [None] + [V[q][:, 128:] for q in (1, 2, 3)]
        p = V0 + V4
        m = V0 - V4
        E = [p + A[2], m - B[2], p - A[2], m + B[2]]
        dd = A[1] - A[3]
        ss = B[1] + B[3]
        O = [A[1] + A[3], (dd - ss) * C45, B[3] - B[1], (dd + ss) * (-C45)]
        ys.append([E[a] + O[a] for a in range(4)] + [E[a] - O[a] for a in range(4)])
    for a in range(8):
        ob[jj, :, 128 * a:128 * (a + 1)] = _pack_pair(ys[0][a], ys[1][a])


def _kernel(x_ref, c_ref, wq_hbm, wuk_hbm, wuv_hbm, wo_hbm,
            bx_hbm, wr_hbm, wi_hbm, mf0_ref, mft_ref, mi_ref, f_ref, fh_ref,
            o_hbm,
            acc_ref, q_s, k_s, v_s, wq_b, wuk_b, wuv_b, wo_b, sems, ao_b, aosem,
            xb, wr_b, wi_b, wrn, win, xs, us, ob, bsems, osems):
    p = pl.program_id(0)
    slot = p % 2

    def wcopies(pp, sl):
        return [
            pltpu.make_async_copy(wq_hbm.bitcast(U32).at[:, pp, :], wq_b.at[sl], sems.at[0, sl]),
            pltpu.make_async_copy(wuk_hbm.bitcast(U32).at[:, pp, :], wuk_b.at[sl], sems.at[1, sl]),
            pltpu.make_async_copy(wuv_hbm.bitcast(U32).at[:, pp, :], wuv_b.at[sl], sems.at[2, sl]),
            pltpu.make_async_copy(wo_hbm.at[pl.ds(pp * 256, 256), :], wo_b.at[sl], sems.at[3, sl]),
        ]

    def bcopies():
        xc = [pltpu.make_async_copy(bx_hbm.bitcast(U32).at[:, jj, :], xb.at[jj], bsems.at[jj])
              for jj in range(8)]
        wc = [pltpu.make_async_copy(wr_hbm.at[pl.ds(0, 512), pl.ds(128 * t, 128)].bitcast(U32),
                                    wr_b.at[t], bsems.at[12 + t]) for t in range(16)]
        wc += [pltpu.make_async_copy(wi_hbm.at[pl.ds(0, 512), pl.ds(128 * t, 128)].bitcast(U32),
                                     wi_b.at[t], bsems.at[28 + t]) for t in range(16)]
        wc += [pltpu.make_async_copy(wr_hbm.at[pl.ds(512, 1), :], wrn, bsems.at[10]),
               pltpu.make_async_copy(wi_hbm.at[pl.ds(512, 1), :], win, bsems.at[11])]
        return xc, wc

    @pl.when(p == 0)
    def _():
        for cp in wcopies(0, 0):
            cp.start()
        acc_ref[...] = jnp.zeros_like(acc_ref)

    @pl.when(p == 1)
    def _():
        xc, wc = bcopies()
        for c in xc + wc:
            c.start()

    @pl.when(p + 1 < NP)
    def _():
        for cp in wcopies(p + 1, 1 - slot):
            cp.start()

    @pl.when(p < NP)
    def _():
        for cp in wcopies(p, slot):
            cp.wait()
        _att_pair(slot, x_ref, c_ref, acc_ref, q_s, k_s, v_s, wq_b, wuk_b, wuv_b, wo_b)

    @pl.when(p == NP)
    def _():
        ao_b[...] = acc_ref[...].astype(BF).reshape(128, 16, M)
        aoc = pltpu.make_async_copy(ao_b, o_hbm.at[:, :, pl.ds(0, 1024)], aosem)
        xc, wc = bcopies()
        for c in xc:
            c.wait()
        lax.fori_loop(0, 8, lambda jj, c: (_b_fwd(jj, xb, mf0_ref, mft_ref, f_ref, xs), c)[1], 0)
        for c in wc:
            c.wait()
        _b_mid(xs, us, wr_b, wi_b, wrn, win)

        def ocopy(jj):
            return pltpu.make_async_copy(ob.at[jj], o_hbm.bitcast(U32).at[:, jj, pl.ds(1024, 1024)],
                                         osems.at[jj])

        def inv_body(jj, c):
            _b_inv(jj, us, fh_ref, mi_ref, ob)
            ocopy(jj).start()
            return c

        aoc.start()
        lax.fori_loop(0, 8, inv_body, 0)
        for jj in range(8):
            ocopy(jj).wait()
        aoc.wait()


@jax.jit
def pallas_concat_heads__compressed_kv_cla__spectral_gfnet__prompt_kernel(
    A_x: jax.Array,
    A_c_kv: jax.Array,
    A_w_q: jax.Array,
    A_w_uk: jax.Array,
    A_w_uv: jax.Array,
    A_w_o: jax.Array,
    B_x: jax.Array,
    B_w_r: jax.Array,
    B_w_i: jax.Array,
):
    Mf0, MfT, Mi, F, Fh = _dft_consts()
    V = pltpu.VMEM
    whole = lambda a: pl.BlockSpec(a.shape, lambda p: (0,) * a.ndim, pipeline_mode=pl.Buffered(1))
    ANY = pl.BlockSpec(memory_space=pl.ANY)
    out = pl.pallas_call(
        _kernel,
        grid=(NP + 1,),
        in_specs=[
            pl.BlockSpec((S, M), lambda p: (0, 0), pipeline_mode=pl.Buffered(1)),
            pl.BlockSpec((S, DC), lambda p: (0, 0), pipeline_mode=pl.Buffered(1)),
            ANY, ANY, ANY, ANY, ANY, ANY, ANY,
            whole(Mf0), whole(MfT), whole(Mi), whole(F), whole(Fh),
        ],
        out_specs=ANY,
        out_shape=jax.ShapeDtypeStruct((128, 16, 2048), BF),
        scratch_shapes=[
            V((S, M), F32), V((S, 256), BF), V((S, 256), BF), V((S, 256), BF),
            V((2, M, 128), U32), V((2, DC, 128), U32), V((2, DC, 128), U32),
            V((2, 256, M), BF), pltpu.SemaphoreType.DMA((4, 2)),
            V((128, 16, M), BF), pltpu.SemaphoreType.DMA(()),
            V((8, 128, 1024), U32), V((16, 256, 128), U32), V((16, 256, 128), U32),
            V((1, 2048), BF), V((1, 2048), BF),
            V((16, NR, 256), F32), V((16, NR, 256), BF), V((8, 128, 1024), U32),
            pltpu.SemaphoreType.DMA((44,)), pltpu.SemaphoreType.DMA((8,)),
        ],
        compiler_params=pltpu.CompilerParams(
            vmem_limit_bytes=110 * 2 ** 20, dimension_semantics=("arbitrary",)),
    )(A_x.reshape(S, M), A_c_kv.reshape(S, DC), A_w_q, A_w_uk, A_w_uv, A_w_o.reshape(H * D, M),
      B_x.reshape(128, 16, 1024), B_w_r.T, B_w_i.T, Mf0, MfT, Mi, F, Fh)
    return out.reshape(1, S, 2048)
```

```python
import jax
import jax.numpy as jnp
import ml_dtypes
import numpy as np
from jax import lax
from jax.experimental import pallas as pl
from jax.experimental.pallas import tpu as pltpu

S = 2048
D = 128
M = 1024
DC = 512
H = 32
NP = H // 2
BQ = 256
CK = 512
NR = 528
NH = NR // 2

F32 = jnp.float32
BF = jnp.bfloat16
U32 = jnp.uint32
NT = (((1,), (1,)), ((), ()))
LOG2E = 1.4426950408889634
C45 = float(np.sqrt(0.5))
HI = np.uint32(0xFFFF0000)


def _k1d(q, h):
    if q == 0:
        return 0 if h == 0 else 4
    return q if h == 0 else 8 - q


def _bf(a):
    return np.asarray(a, np.float32).astype(ml_dtypes.bfloat16)


def _packrows(a):
    a = a.view(np.uint16).astype(np.uint32)
    return a[..., 0::2, :] | (a[..., 1::2, :] << 16)


def _dft_consts():
    b = np.arange(128)[:, None]
    k2 = np.arange(64)[None, :]
    Mf = np.zeros((4, 256, 256))
    Mi = np.zeros((4, 256, 256))
    for q in range(4):
        Ta = np.exp(-2j * np.pi * b * (_k1d(q, 0) + 8 * k2) / 1024.0)
        Tb = np.exp(-2j * np.pi * b * (_k1d(q, 1) + 8 * k2) / 1024.0)
        if q == 0:
            Mf[q, :128, 0:64] = Ta.real
            Mf[q, 128:, 64:128] = Tb.real
            Mf[q, :128, 128:192] = Ta.imag
            Mf[q, 128:, 192:256] = Tb.imag
            w = np.full(256, 2.0)
            w[0] = 1.0
            w[128] = 0.0
            Mi[q] = (Mf[q].T * w[:, None]) / 1024.0
        else:
            Mf[q, :128, 0:64] = Ta.real
            Mf[q, 128:, 0:64] = -Ta.imag
            Mf[q, :128, 64:128] = Tb.real
            Mf[q, 128:, 64:128] = Tb.imag
            Mf[q, :128, 128:192] = Ta.imag
            Mf[q, 128:, 128:192] = Ta.real
            Mf[q, :128, 192:256] = Tb.imag
            Mf[q, 128:, 192:256] = -Tb.real
            Mi[q] = Mf[q].T * 2.0 / 1024.0
    MfT = np.transpose(Mf, (0, 2, 1)).copy()
    Ny = np.zeros((16, 256))
    Ny[0, :128] = (-1.0) ** np.arange(128)
    d1 = np.arange(128)[:, None]
    k1 = np.arange(128)[None, :]
    F = np.zeros((16, 128, 384))
    Fh = np.zeros((16, 384, 128))
    for d2 in range(16):
        f = np.exp(-2j * np.pi * (d1 * k1 / 128.0 + d2 * k1 / 2048.0))
        F[d2] = np.concatenate([f.real, f.real + f.imag, f.imag - f.real], axis=1)
        h = np.conj(f) / 2048.0
        Fh[d2] = np.concatenate([h.real, h.real + h.imag, h.imag - h.real], axis=0)
    Mf0 = np.concatenate([MfT[0], Ny], axis=0)
    return tuple(_packrows(_bf(a)) for a in (Mf0, MfT, Mi, F, Fh))


def _lo(a):
    return pltpu.bitcast(a << 16, F32)


def _hi(a):
    return pltpu.bitcast(a & HI, F32)


def _tb(a):
    return pltpu.bitcast(a, BF)


def _tu(a):
    return pltpu.bitcast(a, U32)


def _tilered(s, op):
    m = s[:, :128]
    for j in range(1, s.shape[1] // 128):
        m = op(m, s[:, j * 128:(j + 1) * 128])
    return m


def _twiddle(xr, xi, k):
    k %= 16
    if k == 0:
        return xr, xi
    if k == 4:
        return -xi, xr
    if k == 8:
        return -xr, -xi
    if k == 12:
        return xi, -xr
    if k == 2:
        return (xr - xi) * C45, (xr + xi) * C45
    if k == 6:
        return (xr + xi) * (-C45), (xr - xi) * C45
    if k == 10:
        return (xi - xr) * C45, (xr + xi) * (-C45)
    if k == 14:
        return (xr + xi) * C45, (xi - xr) * C45
    c = float(np.cos(2 * np.pi * k / 16))
    s = float(np.sin(2 * np.pi * k / 16))
    return xr * c - xi * s, xr * s + xi * c


def _dft4(a, sign):
    (r0, i0), (r1, i1), (r2, i2), (r3, i3) = a
    sr, si = r0 + r2, i0 + i2
    dr, di = r0 - r2, i0 - i2
    tr, ti = r1 + r3, i1 + i3
    ur, ui = r1 - r3, i1 - i3
    o0 = (sr + tr, si + ti)
    o2 = (sr - tr, si - ti)
    if sign < 0:
        o1 = (dr + ui, di - ur)
        o3 = (dr - ui, di + ur)
    else:
        o1 = (dr - ui, di + ur)
        o3 = (dr + ui, di - ur)
    return [o0, o1, o2, o3]


def _dft16(a, sign):
    t = [[None] * 4 for _ in range(4)]
    for n2 in range(4):
        o = _dft4([a[4 * n1 + n2] for n1 in range(4)], sign)
        for k1 in range(4):
            t[k1][n2] = _twiddle(o[k1][0], o[k1][1], sign * n2 * k1)
    out = [None] * 16
    for k1 in range(4):
        o = _dft4(t[k1], sign)
        for k2 in range(4):
            out[k1 + 4 * k2] = o[k2]
    return out


def _pack_pair(a, b):
    ua = pltpu.bitcast(a.astype(BF).astype(F32), U32)
    ub = pltpu.bitcast(b.astype(BF).astype(F32), U32)
    return (ua >> 16) | (ub & HI)


def _make_proj(wslot, qslot, x_s, c_s, q_s, kv_s, wq_b, wuk_b, wuv_b):
    a = wq_b[wslot]
    wq = jnp.concatenate([_lo(a), _hi(a)], axis=1).astype(BF)
    a = wuk_b[wslot]
    b = wuv_b[wslot]
    wkv = jnp.concatenate([_lo(a), _hi(a), _lo(b), _hi(b)], axis=1).astype(BF)
    qscale = (D ** -0.5) * LOG2E

    def proj(i):
        r = slice(i * BQ // 2, (i + 1) * BQ // 2)
        rq = pl.ds(pl.multiple_of(qslot * (S // 2) + i * BQ // 2, BQ // 2), BQ // 2)
        q = jnp.dot(_tb(x_s[r, :]), wq, preferred_element_type=F32)
        q_s[rq, :] = _tu((q * qscale).astype(BF))
        kv = jnp.dot(_tb(c_s[r, :]), wkv, preferred_element_type=F32)
        kv_s[rq, :] = _tu(kv.astype(BF))

    return proj


def _att(slot, acc_ref, q_s, kv_s, wo_b, fillers, final=None):
    wo = _tb(wo_b[slot])
    n = S // BQ
    rr = lax.broadcasted_iota(jnp.int32, (128, 128), 0)
    cc = lax.broadcasted_iota(jnp.int32, (128, 128), 1)
    tri = cc <= rr
    NEG = -1e30

    def rows(r0, nr):
        return pl.ds(pl.multiple_of(slot * (S // 2) + r0 // 2, 64), nr // 2)

    work = []
    for i in range(n):
        for h in range(2):
            kv = BQ * (i + 1) - 128
            c0 = 0
            while c0 < kv:
                w = min(CK, kv - c0)
                work.append((h, i, "f", c0, w, c0 == 0))
                c0 += w
            work.append((h, i, "b", kv, 128, False))
    G = len(work)

    def qk(g):
        h, i, kind, c0, w, first = work[g]
        hs = slice(h * 128, (h + 1) * 128)
        r1 = (i + 1) * BQ
        kk = _tb(kv_s[rows(c0, w), hs])
        if kind == "f":
            s = lax.dot_general(_tb(q_s[rows(i * BQ, BQ), hs]), kk, NT, preferred_element_type=F32)
            if c0 + w == r1 - 128:
                top = jnp.where(tri, s[:128, w - 128:], NEG)
                lastt = jnp.concatenate([top, s[128:, w - 128:]], axis=0)
                s = jnp.concatenate([s[:, :w - 128], lastt], axis=1) if w > 128 else lastt
            return s
        s = lax.dot_general(_tb(q_s[rows(r1 - 128, 128), hs]), kk, NT, preferred_element_type=F32)
        return jnp.where(tri, s, NEG)

    st = {}
    ctxs = {}

    def chain(l, pp):
        for j in range(pp.shape[1] // 128):
            l = l + pp[:, j * 128:(j + 1) * 128]
        return l

    def smpv(g, s):
        h, i, kind, c0, w, first = work[g]
        vv = _tb(kv_s[rows(c0, w), 256 + h * 128:256 + (h + 1) * 128])
        tmx = _tilered(s, jnp.maximum)
        mc = jnp.max(tmx, axis=1, keepdims=True)
        if kind == "f":
            if first:
                m = mc
                pp = jnp.exp2(s - m)
                l = chain(tmx * 0.0, pp)
                o = jnp.dot(pp.astype(BF), vv, preferred_element_type=F32)
            else:
                m0, l0, o0 = st[(h, i)]
                m = jnp.maximum(m0, mc)
                alpha = jnp.exp2(m0 - m)
                pp = jnp.exp2(s - m)
                l = chain(l0 * alpha, pp)
                o = o0 * alpha + jnp.dot(pp.astype(BF), vv, preferred_element_type=F32)
            st[(h, i)] = (m, l, o)
        else:
            m0, l0, o0 = st.pop((h, i))
            mb = jnp.maximum(m0[128:], mc)
            alpha = jnp.exp2(m0[128:] - mb)
            pp = jnp.exp2(s - mb)
            lb = l0[128:] * alpha + pp
            ob = o0[128:] * alpha + jnp.dot(pp.astype(BF), vv, preferred_element_type=F32)
            l = jnp.concatenate([l0[:128], lb], axis=0)
            o = jnp.concatenate([o0[:128], ob], axis=0)
            lsum = jnp.sum(l, axis=1, keepdims=True)
            r = pltpu.reciprocal(lsum, approx=True)
            r = r * (2.0 - lsum * r)
            ctxs[(h, i)] = o * r

    def op(i):
        ctx = jnp.concatenate([ctxs.pop((h, i)) for h in range(2)], axis=1).astype(BF)
        res = jnp.dot(ctx, wo, preferred_element_type=F32)
        if final is None:
            acc_ref[i * BQ:(i + 1) * BQ, :] += res
        else:
            final(i, res)

    fillers = list(fillers)
    ss = {0: qk(0)}
    for g in range(G):
        if g + 1 < G:
            ss[g + 1] = qk(g + 1)
        smpv(g, ss.pop(g))
        h, i, kind = work[g][:3]
        if kind == "b" and h == 1:
            if fillers:
                fillers.pop(0)()
            op(i)


def _b_fwd_d(d2, xb, mf0_ref, mft_ref):
    sel = _lo if d2 % 2 == 0 else _hi
    xa = [sel(xb[d2 // 2, :, 128 * a:128 * (a + 1)]) for a in range(8)]
    u = [xa[a] - xa[a + 4] for a in range(4)]
    ee = [xa[a] + xa[a + 4] for a in range(4)]
    t0 = ee[0] + ee[2]
    t1 = ee[1] + ee[3]
    d = (u[1] - u[3]) * C45
    s = (u[1] + u[3]) * C45
    ins = [(t0 + t1, t0 - t1), (u[0] + d, -(u[2] + s)), (ee[0] - ee[2], ee[3] - ee[1]), (u[0] - d, u[2] - s)]
    zr = []
    zi = []
    for q in range(4):
        r = jnp.concatenate(ins[q], axis=1).astype(BF)
        lhs = _tb(mf0_ref[...] if q == 0 else mft_ref[q])
        z = lax.dot_general(lhs, r, NT, preferred_element_type=F32)
        zr.append(z[:128])
        zi.append(z[128:256])
        if q == 0:
            ny = z[256:272]
    return jnp.concatenate(zr + [ny], axis=0), jnp.concatenate(zi + [jnp.zeros((16, 128), F32)], axis=0)


def _b_fwd_s(d2, zr, zi, f_ref, xs):
    for a, b in ((0, 256), (256, NR)):
        t1 = jnp.dot((zr[a:b] + zi[a:b]).astype(BF), _tb(f_ref[d2, :, 0:128]), preferred_element_type=F32)
        t2 = jnp.dot(zi[a:b].astype(BF), _tb(f_ref[d2, :, 128:256]), preferred_element_type=F32)
        t3 = jnp.dot(zr[a:b].astype(BF), _tb(f_ref[d2, :, 256:384]), preferred_element_type=F32)
        xs[d2, a:b, 0:128] = t1 - t2
        xs[d2, a:b, 128:256] = t1 + t3


def _b_fwd(xb, mf0_ref, mft_ref, f_ref, xs):
    prev = None
    for d2 in range(16):
        cur = _b_fwd_d(d2, xb, mf0_ref, mft_ref)
        if prev is not None:
            _b_fwd_s(d2 - 1, *prev, f_ref, xs)
        prev = cur
    _b_fwd_s(15, *prev, f_ref, xs)


def _b_mid_group(r0, wsel, xs, us):
    r = slice(r0, r0 + 16)
    X = _dft16([(xs[d, r, 0:128], xs[d, r, 128:256]) for d in range(16)], -1)
    Y = []
    for k2 in range(16):
        wr, wi = wsel(k2)
        xr, xi = X[k2]
        Y.append((xr * wr - xi * wi, xr * wi + xi * wr))
    U = _dft16(Y, +1)
    for d in range(16):
        us[NH * d + r0 // 2:NH * d + r0 // 2 + 8, :] = _tu(jnp.concatenate(U[d], axis=1).astype(BF))


def _b_mid(xs, us, wr_b, wi_b, wrn, win):
    for q in range(4):
        for h in range(2):
            kk = _k1d(q, h)
            sel = _lo if kk % 2 == 0 else _hi
            for gg in range(4):
                rows = pl.ds(kk // 2 + 64 * gg, 16, stride=4)
                _b_mid_group(128 * q + 64 * h + 16 * gg,
                             lambda k2: (sel(wr_b[k2, rows, :]), sel(wi_b[k2, rows, :])), xs, us)
    _b_mid_group(
        512,
        lambda k2: (jnp.broadcast_to(wrn[0:1, 128 * k2:128 * (k2 + 1)].astype(F32), (16, 128)),
                    jnp.broadcast_to(win[0:1, 128 * k2:128 * (k2 + 1)].astype(F32), (16, 128))),
        xs, us)


def _b_inv_s(d2, us, fh_ref):
    def parts(r0, nr):
        r = slice(NH * d2 + r0 // 2, NH * d2 + (r0 + nr) // 2)
        ur = _tb(us[r, 0:128])
        ui = _tb(us[r, 128:256])
        return ur, ui, (ur.astype(F32) + ui.astype(F32)).astype(BF)

    h1 = _tb(fh_ref[d2, 0:64, :])
    h2 = _tb(fh_ref[d2, 64:128, :])
    h3 = _tb(fh_ref[d2, 128:192, :])
    out = []
    for q in range(4):
        ur, ui, usum = parts(128 * q, 128)
        t1 = lax.dot_general(h1, usum, NT, preferred_element_type=F32)
        t2 = lax.dot_general(h2, ui, NT, preferred_element_type=F32)
        t3 = lax.dot_general(h3, ur, NT, preferred_element_type=F32)
        out.append(jnp.concatenate([t1 - t2, t1 + t3], axis=1).astype(BF))
    ur, ui, usum = parts(512, 16)
    on = (lax.dot_general(h1, usum, NT, preferred_element_type=F32)
          - lax.dot_general(h2, ui, NT, preferred_element_type=F32))
    return out, on[:, 0:1]


def _b_inv_d(lhs, ny, mi_ref):
    sgn = jnp.where(lax.broadcasted_iota(jnp.int32, (128, 128), 1) % 2 == 0,
                    1.0 / 1024, -1.0 / 1024).astype(F32)
    V = [jnp.dot(lhs[q], _tb(mi_ref[q]), preferred_element_type=F32) for q in range(4)]
    V0 = V[0][:, :128] + ny * sgn
    V4 = V[0][:, 128:]
    A = [None] + [V[q][:, :128] for q in (1, 2, 3)]
    B = [None] + [V[q][:, 128:] for q in (1, 2, 3)]
    p = V0 + V4
    m = V0 - V4
    E = [p + A[2], m - B[2], p - A[2], m + B[2]]
    dd = A[1] - A[3]
    ss = B[1] + B[3]
    O = [A[1] + A[3], (dd - ss) * C45, B[3] - B[1], (dd + ss) * (-C45)]
    return [E[a] + O[a] for a in range(4)] + [E[a] - O[a] for a in range(4)]


def _b_inv(jjs, us, fh_ref, mi_ref, ob):
    ys = {}

    def fin(d2, lh):
        ys[d2] = _b_inv_d(*lh, mi_ref)
        if d2 % 2 == 1:
            for a in range(8):
                ob[d2 // 2, :, 128 * a:128 * (a + 1)] = _pack_pair(ys[d2 - 1][a], ys[d2][a])
            del ys[d2 - 1], ys[d2]

    prev = None
    for d2 in [2 * jj + e for jj in jjs for e in range(2)]:
        cur = _b_inv_s(d2, us, fh_ref)
        if prev is not None:
            fin(*prev)
        prev = (d2, cur)
    fin(*prev)


def _kernel(x_hbm, c_hbm, wq_hbm, wuk_hbm, wuv_hbm, wo_hbm, bx_hbm, wr_hbm, wi_hbm,
            mf0_hbm, mft_hbm, mi_hbm, f_hbm, fh_hbm,
            o_hbm,
            x_s, c_s, acc_ref, q_s, kv_s, wq_b, wuk_b, wuv_b, wo_b, ao_b,
            xb, wr_b, wi_b, wrn, win, mf0_ref, mft_ref, mi_ref, f_ref, fh_ref, xs, us, ob,
            wsem, isem, xsem, wrsem, osem, asem):
    cp = pltpu.make_async_copy

    def pcopies(pp, sl):
        return [cp(wq_hbm.bitcast(U32).at[:, pp, :], wq_b.at[sl], wsem.at[0, sl]),
                cp(wuk_hbm.bitcast(U32).at[:, pp, :], wuk_b.at[sl], wsem.at[1, sl]),
                cp(wuv_hbm.bitcast(U32).at[:, pp, :], wuv_b.at[sl], wsem.at[2, sl])]

    def ocopy(pp, sl):
        return cp(wo_hbm.bitcast(U32).at[pl.ds(pp * 128, 128), :], wo_b.at[sl], wsem.at[3, sl])

    bcopies = [cp(mf0_hbm, mf0_ref, isem.at[0]), cp(mft_hbm, mft_ref, isem.at[1]), cp(f_hbm, f_ref, isem.at[2]),
               cp(mi_hbm, mi_ref, isem.at[3]), cp(fh_hbm, fh_ref, isem.at[4])]
    bcopies += [cp(bx_hbm.bitcast(U32).at[:, jj, :], xb.at[jj], xsem.at[jj]) for jj in range(8)]
    bcopies += [cp(wr_hbm.at[pl.ds(0, 512), pl.ds(128 * t, 128)].bitcast(U32), wr_b.at[t], wrsem.at[t])
                for t in range(16)]
    bcopies += [cp(wi_hbm.at[pl.ds(0, 512), pl.ds(128 * t, 128)].bitcast(U32), wi_b.at[t], wrsem.at[16 + t])
                for t in range(16)]
    bcopies += [cp(wr_hbm.at[pl.ds(512, 1), :], wrn, wrsem.at[32]),
                cp(wi_hbm.at[pl.ds(512, 1), :], win, wrsem.at[33])]
    acopies = [(cp(x_hbm.bitcast(U32).at[pl.ds(128 * i, 128), :], x_s.at[pl.ds(128 * i, 128), :], asem.at[0, i]),
                cp(c_hbm.bitcast(U32).at[pl.ds(128 * i, 128), :], c_s.at[pl.ds(128 * i, 128), :], asem.at[1, i]))
               for i in range(8)]

    for c in pcopies(0, 0) + list(acopies[0]):
        c.start()
    acc_ref[...] = jnp.zeros_like(acc_ref)
    for c in pcopies(0, 0):
        c.wait()
    proj0 = _make_proj(0, 0, x_s, c_s, q_s, kv_s, wq_b, wuk_b, wuv_b)
    for i in range(8):
        for c in acopies[i]:
            c.wait()
        for j in ((1, 2) if i == 0 else (i + 2,)):
            if j < 8:
                for c in acopies[j]:
                    c.start()
            if j == 7:
                for c in pcopies(1, 1) + [ocopy(0, 0)]:
                    c.start()
        proj0(i)
    for c in bcopies:
        c.start()

    def step(p, carry):
        slot = p % 2
        for c in pcopies(p + 1, 1 - slot) + [ocopy(p, slot)]:
            c.wait()
        ocopy(p + 1, 1 - slot).start()

        @pl.when(p + 2 < NP)
        def _():
            for c in pcopies(p + 2, slot):
                c.start()

        proj = _make_proj(1 - slot, 1 - slot, x_s, c_s, q_s, kv_s, wq_b, wuk_b, wuv_b)
        _att(slot, acc_ref, q_s, kv_s, wo_b, [(lambda i=i: proj(i)) for i in range(8)])
        return carry

    lax.fori_loop(0, NP - 1, step, 0)

    ocopy(NP - 1, 1).wait()
    for c in bcopies:
        c.wait()

    def final(i, res):
        ao_b[16 * i:16 * (i + 1)] = (acc_ref[i * BQ:(i + 1) * BQ, :] + res).astype(BF).reshape(16, 16, M)

    _att(1, acc_ref, q_s, kv_s, wo_b, [], final=final)
    aoc = cp(ao_b, o_hbm.at[:, :, pl.ds(0, 1024)], isem.at[5])
    aoc.start()
    _b_fwd(xb, mf0_ref, mft_ref, f_ref, xs)
    _b_mid(xs, us, wr_b, wi_b, wrn, win)
    ocs = [cp(ob.at[jj], o_hbm.bitcast(U32).at[:, jj, pl.ds(1024, 1024)], osem.at[jj]) for jj in range(8)]
    for grp in ((0, 1, 2, 3, 4), (5, 6), (7,)):
        _b_inv(grp, us, fh_ref, mi_ref, ob)
        for jj in grp:
            ocs[jj].start()
    for c in ocs:
        c.wait()
    aoc.wait()


@jax.jit
def pallas_concat_heads__compressed_kv_cla__spectral_gfnet__prompt_kernel(
    A_x: jax.Array,
    A_c_kv: jax.Array,
    A_w_q: jax.Array,
    A_w_uk: jax.Array,
    A_w_uv: jax.Array,
    A_w_o: jax.Array,
    B_x: jax.Array,
    B_w_r: jax.Array,
    B_w_i: jax.Array,
):
    Mf0, MfT, Mi, F, Fh = _dft_consts()
    V = pltpu.VMEM
    SD = pltpu.SemaphoreType.DMA
    ANY = pl.BlockSpec(memory_space=pl.ANY)
    out = pl.pallas_call(
        _kernel,
        in_specs=[ANY] * 14,
        out_specs=ANY,
        out_shape=jax.ShapeDtypeStruct((128, 16, 2048), BF),
        scratch_shapes=[
            V((S // 2, M), U32), V((S // 2, DC), U32), V((S, M), F32), V((S, 256), U32), V((S, 512), U32),
            V((2, M, 128), U32), V((2, DC, 128), U32), V((2, DC, 128), U32), V((2, 128, M), U32),
            V((128, 16, M), BF),
            V((8, 128, 1024), U32), V((16, 256, 128), U32), V((16, 256, 128), U32),
            V((1, 2048), BF), V((1, 2048), BF),
            V(Mf0.shape, U32), V(MfT.shape, U32), V(Mi.shape, U32), V(F.shape, U32), V(Fh.shape, U32),
            V((16, NR, 256), F32), V((16 * NH, 256), U32), V((8, 128, 1024), U32),
            SD((4, 2)), SD((6,)), SD((8,)), SD((34,)), SD((8,)), SD((2, 8)),
        ],
        compiler_params=pltpu.CompilerParams(vmem_limit_bytes=120 * 2 ** 20, disable_bounds_checks=True),
    )(A_x.reshape(S, M), A_c_kv.reshape(S, DC), A_w_q, A_w_uk, A_w_uv, A_w_o.reshape(H * D, M),
      B_x.reshape(128, 16, 1024), B_w_r.T, B_w_i.T, Mf0, MfT, Mi, F, Fh)
    return out.reshape(1, S, 2048)
```

```python
import jax
import jax.numpy as jnp
import ml_dtypes
import numpy as np
from jax import lax
from jax.experimental import pallas as pl
from jax.experimental.pallas import tpu as pltpu

S = 2048
D = 128
M = 1024
DC = 512
H = 32
NP = H // 2
BQ = 256
NR = 528
NH = NR // 2

LOOP_PLAN = dict(order=(5, 2, 4, 1, 3, 0, 6, 7), ck=512, chain=False, split_op=True,
                 opd=(0, 0, 0, 0, 0, 0, 0, 3), opd2=(3, 1, 1, 0, 1, 0, 3, 0),
                 fpos=(0, 8, 14, 23, 28, 33, 50, 52))
LAST_PLAN = dict(order=(6, 3, 0, 2, 1, 5, 7, 4), ck=384, chain=True, split_op=False,
                 opd=(0, 0, 2, 0, 3, 0, 0, 0), opd2=None, fpos=None)

F32 = jnp.float32
BF = jnp.bfloat16
U32 = jnp.uint32
NT = (((1,), (1,)), ((), ()))
LOG2E = 1.4426950408889634
C45 = float(np.sqrt(0.5))
HI = np.uint32(0xFFFF0000)


def _k1d(q, h):
    if q == 0:
        return 0 if h == 0 else 4
    return q if h == 0 else 8 - q


def _bf(a):
    return np.asarray(a, np.float32).astype(ml_dtypes.bfloat16)


def _packrows(a):
    a = a.view(np.uint16).astype(np.uint32)
    return a[..., 0::2, :] | (a[..., 1::2, :] << 16)


def _dft_consts():
    b = np.arange(128)[:, None]
    k2 = np.arange(64)[None, :]
    Mf = np.zeros((4, 256, 256))
    Mi = np.zeros((4, 256, 256))
    for q in range(4):
        Ta = np.exp(-2j * np.pi * b * (_k1d(q, 0) + 8 * k2) / 1024.0)
        Tb = np.exp(-2j * np.pi * b * (_k1d(q, 1) + 8 * k2) / 1024.0)
        if q == 0:
            Mf[q, :128, 0:64] = Ta.real
            Mf[q, 128:, 64:128] = Tb.real
            Mf[q, :128, 128:192] = Ta.imag
            Mf[q, 128:, 192:256] = Tb.imag
            w = np.full(256, 2.0)
            w[0] = 1.0
            w[128] = 0.0
            Mi[q] = (Mf[q].T * w[:, None]) / 1024.0
        else:
            Mf[q, :128, 0:64] = Ta.real
            Mf[q, 128:, 0:64] = -Ta.imag
            Mf[q, :128, 64:128] = Tb.real
            Mf[q, 128:, 64:128] = Tb.imag
            Mf[q, :128, 128:192] = Ta.imag
            Mf[q, 128:, 128:192] = Ta.real
            Mf[q, :128, 192:256] = Tb.imag
            Mf[q, 128:, 192:256] = -Tb.real
            Mi[q] = Mf[q].T * 2.0 / 1024.0
    Mi[0, 128, :128] = ((-1.0) ** np.arange(128)) / 1024.0
    MfT = np.transpose(Mf, (0, 2, 1)).copy()
    Ny = np.zeros((16, 256))
    Ny[0, :128] = (-1.0) ** np.arange(128)
    d1 = np.arange(128)[:, None]
    k1 = np.arange(128)[None, :]
    F = np.zeros((16, 128, 384))
    Fh = np.zeros((16, 384, 128))
    for d2 in range(16):
        f = np.exp(-2j * np.pi * (d1 * k1 / 128.0 + d2 * k1 / 2048.0))
        F[d2] = np.concatenate([f.real, f.real + f.imag, f.imag - f.real], axis=1)
        h = np.conj(f) / 2048.0
        Fh[d2] = np.concatenate([h.real, h.real + h.imag, h.imag - h.real], axis=0)
    Mf0 = np.concatenate([MfT[0], Ny], axis=0)
    return tuple(_packrows(_bf(a)) for a in (Mf0, MfT, Mi, F, Fh))


def _lo(a):
    return pltpu.bitcast(a << 16, F32)


def _hi(a):
    return pltpu.bitcast(a & HI, F32)


def _tb(a):
    return pltpu.bitcast(a, BF)


def _tu(a):
    return pltpu.bitcast(a, U32)


def _tilered(s, op):
    m = s[:, :128]
    for j in range(1, s.shape[1] // 128):
        m = op(m, s[:, j * 128:(j + 1) * 128])
    return m


def _twiddle(xr, xi, k):
    k %= 16
    if k == 0:
        return xr, xi
    if k == 4:
        return -xi, xr
    if k == 8:
        return -xr, -xi
    if k == 12:
        return xi, -xr
    if k == 2:
        return (xr - xi) * C45, (xr + xi) * C45
    if k == 6:
        return (xr + xi) * (-C45), (xr - xi) * C45
    if k == 10:
        return (xi - xr) * C45, (xr + xi) * (-C45)
    if k == 14:
        return (xr + xi) * C45, (xi - xr) * C45
    c = float(np.cos(2 * np.pi * k / 16))
    s = float(np.sin(2 * np.pi * k / 16))
    return xr * c - xi * s, xr * s + xi * c


def _dft4(a, sign):
    (r0, i0), (r1, i1), (r2, i2), (r3, i3) = a
    sr, si = r0 + r2, i0 + i2
    dr, di = r0 - r2, i0 - i2
    tr, ti = r1 + r3, i1 + i3
    ur, ui = r1 - r3, i1 - i3
    o0 = (sr + tr, si + ti)
    o2 = (sr - tr, si - ti)
    if sign < 0:
        o1 = (dr + ui, di - ur)
        o3 = (dr - ui, di + ur)
    else:
        o1 = (dr - ui, di + ur)
        o3 = (dr + ui, di - ur)
    return [o0, o1, o2, o3]


def _dft16(a, sign):
    t = [[None] * 4 for _ in range(4)]
    for n2 in range(4):
        o = _dft4([a[4 * n1 + n2] for n1 in range(4)], sign)
        for k1 in range(4):
            t[k1][n2] = _twiddle(o[k1][0], o[k1][1], sign * n2 * k1)
    out = [None] * 16
    for k1 in range(4):
        o = _dft4(t[k1], sign)
        for k2 in range(4):
            out[k1 + 4 * k2] = o[k2]
    return out


def _pack_pair(a, b):
    ua = pltpu.bitcast(a.astype(BF).astype(F32), U32)
    ub = pltpu.bitcast(b.astype(BF).astype(F32), U32)
    return (ua >> 16) | (ub & HI)


def _make_proj(wslot, qslot, x_s, c_s, q_s, kv_s, wq_b, wuk_b, wuv_b):
    a = wq_b[wslot]
    wq = jnp.concatenate([_lo(a), _hi(a)], axis=1).astype(BF)
    a = wuk_b[wslot]
    b = wuv_b[wslot]
    wkv = jnp.concatenate([_lo(a), _hi(a), _lo(b), _hi(b)], axis=1).astype(BF)
    qscale = (D ** -0.5) * LOG2E

    def proj(i):
        r = slice(i * BQ // 2, (i + 1) * BQ // 2)
        rq = pl.ds(pl.multiple_of(qslot * (S // 2) + i * BQ // 2, BQ // 2), BQ // 2)
        q = jnp.dot(_tb(x_s[r, :]), wq, preferred_element_type=F32)
        q_s[rq, :] = _tu((q * qscale).astype(BF))
        kv = jnp.dot(_tb(c_s[r, :]), wkv, preferred_element_type=F32)
        kv_s[rq, :] = _tu(kv.astype(BF))

    return proj


def _att(slot, acc_ref, q_s, kv_s, wo_b, fillers, plan, final=None):
    wo = _tb(wo_b[slot])
    n = S // BQ
    rr = lax.broadcasted_iota(jnp.int32, (128, 128), 0)
    cc = lax.broadcasted_iota(jnp.int32, (128, 128), 1)
    tri = cc <= rr
    NEG = -1e30

    def rows(r0, nr):
        return pl.ds(pl.multiple_of(slot * (S // 2) + r0 // 2, 64), nr // 2)

    work = []
    CK = plan["ck"]
    order = plan["order"]
    for i in order:
        for h in range(2):
            kv = BQ * (i + 1) - 128
            c0 = 0
            while c0 < kv:
                w = min(CK, kv - c0)
                work.append((h, i, "f", c0, w, c0 == 0))
                c0 += w
            work.append((h, i, "b", kv, 128, False))
    G = len(work)

    def qk(g):
        h, i, kind, c0, w, first = work[g]
        hs = slice(h * 128, (h + 1) * 128)
        r1 = (i + 1) * BQ
        kk = _tb(kv_s[rows(c0, w), hs])
        if kind == "f":
            s = lax.dot_general(_tb(q_s[rows(i * BQ, BQ), hs]), kk, NT, preferred_element_type=F32)
            if c0 + w == r1 - 128:
                top = jnp.where(tri, s[:128, w - 128:], NEG)
                lastt = jnp.concatenate([top, s[128:, w - 128:]], axis=0)
                s = jnp.concatenate([s[:, :w - 128], lastt], axis=1) if w > 128 else lastt
            return s
        s = lax.dot_general(_tb(q_s[rows(r1 - 128, 128), hs]), kk, NT, preferred_element_type=F32)
        return jnp.where(tri, s, NEG)

    st = {}
    ctxs = {}

    def chain(l, pp):
        if not plan["chain"]:
            return l + _tilered(pp, jnp.add)
        for j in range(pp.shape[1] // 128):
            l = l + pp[:, j * 128:(j + 1) * 128]
        return l

    def smpv(g, s):
        h, i, kind, c0, w, first = work[g]
        vv = _tb(kv_s[rows(c0, w), 256 + h * 128:256 + (h + 1) * 128])
        tmx = _tilered(s, jnp.maximum)
        mc = jnp.max(tmx, axis=1, keepdims=True)
        if kind == "f":
            if first:
                m = mc
                pp = jnp.exp2(s - m)
                l = chain(tmx * 0.0, pp) if plan["chain"] else _tilered(pp, jnp.add)
                o = jnp.dot(pp.astype(BF), vv, preferred_element_type=F32)
            else:
                m0, l0, o0 = st[(h, i)]
                m = jnp.maximum(m0, mc)
                alpha = jnp.exp2(m0 - m)
                pp = jnp.exp2(s - m)
                l = chain(l0 * alpha, pp)
                o = o0 * alpha + jnp.dot(pp.astype(BF), vv, preferred_element_type=F32)
            st[(h, i)] = (m, l, o)
        else:
            m0, l0, o0 = st.pop((h, i))
            mb = jnp.maximum(m0[128:], mc)
            alpha = jnp.exp2(m0[128:] - mb)
            pp = jnp.exp2(s - mb)
            lb = l0[128:] * alpha + pp
            ob = o0[128:] * alpha + jnp.dot(pp.astype(BF), vv, preferred_element_type=F32)
            l = jnp.concatenate([l0[:128], lb], axis=0)
            o = jnp.concatenate([o0[:128], ob], axis=0)
            lsum = jnp.sum(l, axis=1, keepdims=True)
            r = pltpu.reciprocal(lsum, approx=True)
            r = r * (2.0 - lsum * r)
            ctxs[(h, i)] = o * r

    def op(i, half):
        ctx = jnp.concatenate([ctxs[(h, i)] for h in range(2)], axis=1).astype(BF)
        cs = slice(0, M) if half is None else slice(half * 512, half * 512 + 512)
        res = jnp.dot(ctx, wo[:, cs], preferred_element_type=F32)
        if final is None:
            acc_ref[i * BQ:(i + 1) * BQ, cs] += res
        else:
            final(i, res)

    done_at = {}
    for g, (h, i, kind, c0, w, first) in enumerate(work):
        if kind == "b" and h == 1:
            done_at[i] = g
    extra = {g: [] for g in range(G)}
    for k, i in enumerate(order):
        g = min(G - 1, done_at[i] + plan["opd"][k])
        if plan["split_op"]:
            extra[g].append((1, lambda i=i: op(i, 0)))
            extra[min(G - 1, g + plan["opd2"][k])].append((2, lambda i=i: op(i, 1)))
        else:
            extra[g].append((1, lambda i=i: op(i, None)))
    for k, f in enumerate(fillers):
        extra[plan["fpos"][k]].append((3, f))

    ss = {0: qk(0)}
    for g in range(G):
        if g + 1 < G:
            ss[g + 1] = qk(g + 1)
        smpv(g, ss.pop(g))
        for _, f in sorted(extra[g], key=lambda t: t[0]):
            f()


def _b_fwd_d(d2, xb, mf0_ref, mft_ref):
    sel = _lo if d2 % 2 == 0 else _hi
    xa = [sel(xb[d2 // 2, :, 128 * a:128 * (a + 1)]) for a in range(8)]
    u = [xa[a] - xa[a + 4] for a in range(4)]
    ee = [xa[a] + xa[a + 4] for a in range(4)]
    t0 = ee[0] + ee[2]
    t1 = ee[1] + ee[3]
    d = (u[1] - u[3]) * C45
    s = (u[1] + u[3]) * C45
    ins = [(t0 + t1, t0 - t1), (u[0] + d, -(u[2] + s)), (ee[0] - ee[2], ee[3] - ee[1]), (u[0] - d, u[2] - s)]
    zr = []
    zi = []
    for q in range(4):
        r = jnp.concatenate(ins[q], axis=1).astype(BF)
        lhs = _tb(mf0_ref[...] if q == 0 else mft_ref[q])
        z = lax.dot_general(lhs, r, NT, preferred_element_type=F32)
        zr.append(z[:128])
        zi.append(z[128:256])
        if q == 0:
            ny = z[256:272]
    return jnp.concatenate(zr + [ny], axis=0), jnp.concatenate(zi + [jnp.zeros((16, 128), F32)], axis=0)


def _b_fwd_s(d2, zr, zi, f_ref, xs):
    for a, b in ((0, 256), (256, NR)):
        t1 = jnp.dot((zr[a:b] + zi[a:b]).astype(BF), _tb(f_ref[d2, :, 0:128]), preferred_element_type=F32)
        t2 = jnp.dot(zi[a:b].astype(BF), _tb(f_ref[d2, :, 128:256]), preferred_element_type=F32)
        t3 = jnp.dot(zr[a:b].astype(BF), _tb(f_ref[d2, :, 256:384]), preferred_element_type=F32)
        xs[d2, a:b, 0:128] = t1 - t2
        xs[d2, a:b, 128:256] = t1 + t3


def _b_fwd(xb, mf0_ref, mft_ref, f_ref, xs):
    prev = None
    for d2 in range(16):
        cur = _b_fwd_d(d2, xb, mf0_ref, mft_ref)
        if prev is not None:
            _b_fwd_s(d2 - 1, *prev, f_ref, xs)
        prev = cur
    _b_fwd_s(15, *prev, f_ref, xs)


def _b_mid_group(r0, wsel, xs, us):
    r = slice(r0, r0 + 16)
    X = _dft16([(xs[d, r, 0:128], xs[d, r, 128:256]) for d in range(16)], -1)
    Y = []
    for k2 in range(16):
        wr, wi = wsel(k2)
        xr, xi = X[k2]
        Y.append((xr * wr - xi * wi, xr * wi + xi * wr))
    U = _dft16(Y, +1)
    for d in range(16):
        us[NH * d + r0 // 2:NH * d + r0 // 2 + 8, :] = _tu(jnp.concatenate(U[d], axis=1).astype(BF))


def _b_mid(xs, us, wr_b, wi_b, wrn, win):
    for q in range(4):
        for h in range(2):
            kk = _k1d(q, h)
            sel = _lo if kk % 2 == 0 else _hi
            for gg in range(4):
                rows = pl.ds(kk // 2 + 64 * gg, 16, stride=4)
                _b_mid_group(128 * q + 64 * h + 16 * gg,
                             lambda k2: (sel(wr_b[k2, rows, :]), sel(wi_b[k2, rows, :])), xs, us)
    _b_mid_group(
        512,
        lambda k2: (jnp.broadcast_to(wrn[0:1, 128 * k2:128 * (k2 + 1)].astype(F32), (16, 128)),
                    jnp.broadcast_to(win[0:1, 128 * k2:128 * (k2 + 1)].astype(F32), (16, 128))),
        xs, us)


def _b_inv_s(jj, us, fh_ref):
    lane = lax.broadcasted_iota(jnp.int32, (128, 128), 1)

    def parts(d2, r0, nr):
        r = slice(NH * d2 + r0 // 2, NH * d2 + (r0 + nr) // 2)
        ur = _tb(us[r, 0:128])
        ui = _tb(us[r, 128:256])
        return ur, ui, (ur.astype(F32) + ui.astype(F32)).astype(BF)

    hs = [[_tb(fh_ref[2 * jj + e, 64 * k:64 * k + 64, :]) for k in range(3)] for e in range(2)]
    out = []
    for q in range(4):
        uu = []
        for e in range(2):
            h1, h2, h3 = hs[e]
            ur, ui, usum = parts(2 * jj + e, 128 * q, 128)
            t1 = lax.dot_general(h1, usum, NT, preferred_element_type=F32)
            t2 = lax.dot_general(h2, ui, NT, preferred_element_type=F32)
            t3 = lax.dot_general(h3, ur, NT, preferred_element_type=F32)
            re = t1 - t2
            im = t1 + t3
            if q == 0:
                _, ni, nsum = parts(2 * jj + e, 512, 16)
                on = (lax.dot_general(h1, nsum, NT, preferred_element_type=F32)
                      - lax.dot_general(h2, ni, NT, preferred_element_type=F32))
                im = jnp.where(lane == 0, jnp.broadcast_to(on[:, 0:1], (128, 128)), im)
            uu.append(jnp.concatenate([re, im], axis=1))
        out.append(_tb(_pack_pair(uu[0], uu[1])))
    return out


def _b_inv_d(jj, lhs, mi_ref, ob):
    V = [jnp.dot(lhs[q], _tb(mi_ref[q]), preferred_element_type=F32) for q in range(4)]
    V0 = V[0][:, :128]
    V4 = V[0][:, 128:]
    A = [None] + [V[q][:, :128] for q in (1, 2, 3)]
    B = [None] + [V[q][:, 128:] for q in (1, 2, 3)]
    p = V0 + V4
    m = V0 - V4
    E = [p + A[2], m - B[2], p - A[2], m + B[2]]
    dd = A[1] - A[3]
    ss = B[1] + B[3]
    O = [A[1] + A[3], (dd - ss) * C45, B[3] - B[1], (dd + ss) * (-C45)]
    ys = [E[a] + O[a] for a in range(4)] + [E[a] - O[a] for a in range(4)]
    ob[jj] = _tu(jnp.concatenate(ys, axis=1).astype(BF))


def _b_inv(jjs, us, fh_ref, mi_ref, ob):
    prev = None
    for jj in jjs:
        cur = _b_inv_s(jj, us, fh_ref)
        if prev is not None:
            _b_inv_d(*prev, mi_ref, ob)
        prev = (jj, cur)
    _b_inv_d(*prev, mi_ref, ob)


def _kernel(x_hbm, c_hbm, wq_hbm, wuk_hbm, wuv_hbm, wo_hbm, bx_hbm, wr_hbm, wi_hbm,
            mf0_hbm, mft_hbm, mi_hbm, f_hbm, fh_hbm,
            o_hbm,
            x_s, c_s, acc_ref, q_s, kv_s, wq_b, wuk_b, wuv_b, wo_b, ao_b,
            xb, wr_b, wi_b, wrn, win, mf0_ref, mft_ref, mi_ref, f_ref, fh_ref, xs, us, ob,
            wsem, isem, xsem, wrsem, osem, asem):
    cp = pltpu.make_async_copy

    def pcopies(pp, sl):
        return [cp(wq_hbm.bitcast(U32).at[:, pp, :], wq_b.at[sl], wsem.at[0, sl]),
                cp(wuk_hbm.bitcast(U32).at[:, pp, :], wuk_b.at[sl], wsem.at[1, sl]),
                cp(wuv_hbm.bitcast(U32).at[:, pp, :], wuv_b.at[sl], wsem.at[2, sl])]

    def ocopy(pp, sl):
        return cp(wo_hbm.bitcast(U32).at[pl.ds(pp * 128, 128), :], wo_b.at[sl], wsem.at[3, sl])

    bcopies = [cp(mf0_hbm, mf0_ref, isem.at[0]), cp(mft_hbm, mft_ref, isem.at[1]), cp(f_hbm, f_ref, isem.at[2]),
               cp(mi_hbm, mi_ref, isem.at[3]), cp(fh_hbm, fh_ref, isem.at[4])]
    bcopies += [cp(bx_hbm.bitcast(U32).at[:, jj, :], xb.at[jj], xsem.at[jj]) for jj in range(8)]
    bcopies += [cp(wr_hbm.at[pl.ds(0, 512), pl.ds(128 * t, 128)].bitcast(U32), wr_b.at[t], wrsem.at[t])
                for t in range(16)]
    bcopies += [cp(wi_hbm.at[pl.ds(0, 512), pl.ds(128 * t, 128)].bitcast(U32), wi_b.at[t], wrsem.at[16 + t])
                for t in range(16)]
    bcopies += [cp(wr_hbm.at[pl.ds(512, 1), :], wrn, wrsem.at[32]),
                cp(wi_hbm.at[pl.ds(512, 1), :], win, wrsem.at[33])]
    acopies = [(cp(x_hbm.bitcast(U32).at[pl.ds(128 * i, 128), :], x_s.at[pl.ds(128 * i, 128), :], asem.at[0, i]),
                cp(c_hbm.bitcast(U32).at[pl.ds(128 * i, 128), :], c_s.at[pl.ds(128 * i, 128), :], asem.at[1, i]))
               for i in range(8)]

    for c in pcopies(0, 0) + list(acopies[0]):
        c.start()
    acc_ref[...] = jnp.zeros_like(acc_ref)
    for c in pcopies(0, 0):
        c.wait()
    proj0 = _make_proj(0, 0, x_s, c_s, q_s, kv_s, wq_b, wuk_b, wuv_b)
    for i in range(8):
        for c in acopies[i]:
            c.wait()
        for j in ((1, 2) if i == 0 else (i + 2,)):
            if j < 8:
                for c in acopies[j]:
                    c.start()
            if j == 7:
                for c in pcopies(1, 1) + [ocopy(0, 0)]:
                    c.start()
        proj0(i)
    for c in bcopies:
        c.start()

    def step(p, carry):
        slot = p % 2
        for c in pcopies(p + 1, 1 - slot) + [ocopy(p, slot)]:
            c.wait()
        ocopy(p + 1, 1 - slot).start()

        @pl.when(p + 2 < NP)
        def _():
            for c in pcopies(p + 2, slot):
                c.start()

        proj = _make_proj(1 - slot, 1 - slot, x_s, c_s, q_s, kv_s, wq_b, wuk_b, wuv_b)
        _att(slot, acc_ref, q_s, kv_s, wo_b, [(lambda i=i: proj(i)) for i in range(8)], LOOP_PLAN)
        return carry

    lax.fori_loop(0, NP - 1, step, 0)

    ocopy(NP - 1, 1).wait()
    for c in bcopies:
        c.wait()

    def final(i, res):
        ao_b[16 * i:16 * (i + 1)] = (acc_ref[i * BQ:(i + 1) * BQ, :] + res).astype(BF).reshape(16, 16, M)

    _att(1, acc_ref, q_s, kv_s, wo_b, [], LAST_PLAN, final=final)
    aoc = cp(ao_b, o_hbm.at[:, :, pl.ds(0, 1024)], isem.at[5])
    aoc.start()
    _b_fwd(xb, mf0_ref, mft_ref, f_ref, xs)
    _b_mid(xs, us, wr_b, wi_b, wrn, win)
    ocs = [cp(ob.at[jj], o_hbm.bitcast(U32).at[:, jj, pl.ds(1024, 1024)], osem.at[jj]) for jj in range(8)]
    for grp in ((0, 1, 2, 3, 4), (5, 6), (7,)):
        _b_inv(grp, us, fh_ref, mi_ref, ob)
        for jj in grp:
            ocs[jj].start()
    for c in ocs:
        c.wait()
    aoc.wait()


@jax.jit
def pallas_concat_heads__compressed_kv_cla__spectral_gfnet__prompt_kernel(
    A_x: jax.Array,
    A_c_kv: jax.Array,
    A_w_q: jax.Array,
    A_w_uk: jax.Array,
    A_w_uv: jax.Array,
    A_w_o: jax.Array,
    B_x: jax.Array,
    B_w_r: jax.Array,
    B_w_i: jax.Array,
):
    Mf0, MfT, Mi, F, Fh = _dft_consts()
    V = pltpu.VMEM
    SD = pltpu.SemaphoreType.DMA
    ANY = pl.BlockSpec(memory_space=pl.ANY)
    out = pl.pallas_call(
        _kernel,
        in_specs=[ANY] * 14,
        out_specs=ANY,
        out_shape=jax.ShapeDtypeStruct((128, 16, 2048), BF),
        scratch_shapes=[
            V((S // 2, M), U32), V((S // 2, DC), U32), V((S, M), F32), V((S, 256), U32), V((S, 512), U32),
            V((2, M, 128), U32), V((2, DC, 128), U32), V((2, DC, 128), U32), V((2, 128, M), U32),
            V((128, 16, M), BF),
            V((8, 128, 1024), U32), V((16, 256, 128), U32), V((16, 256, 128), U32),
            V((1, 2048), BF), V((1, 2048), BF),
            V(Mf0.shape, U32), V(MfT.shape, U32), V(Mi.shape, U32), V(F.shape, U32), V(Fh.shape, U32),
            V((16, NR, 256), F32), V((16 * NH, 256), U32), V((8, 128, 1024), U32),
            SD((4, 2)), SD((6,)), SD((8,)), SD((34,)), SD((8,)), SD((2, 8)),
        ],
        compiler_params=pltpu.CompilerParams(vmem_limit_bytes=120 * 2 ** 20, disable_bounds_checks=True),
    )(A_x.reshape(S, M), A_c_kv.reshape(S, DC), A_w_q, A_w_uk, A_w_uv, A_w_o.reshape(H * D, M),
      B_x.reshape(128, 16, 1024), B_w_r.T, B_w_i.T, Mf0, MfT, Mi, F, Fh)
    return out.reshape(1, S, 2048)
```
